```python
import os as _os
_os.environ.setdefault('JAX_PLATFORMS', 'cpu')
import jax
import jax.numpy as jnp

def _softmax(x, axis=-1):
    return jax.nn.softmax(x, axis=axis)

def _gelu(x):
    return jax.nn.gelu(x, approximate=True)

def _silu(x):
    return jax.nn.silu(x)

def _sigmoid(x):
    return jax.nn.sigmoid(x)

def _layernorm(x, axis=-1, eps=1e-05):
    m = jnp.mean(x, axis=axis, keepdims=True)
    v = jnp.var(x, axis=axis, keepdims=True)
    return (x - m) / jnp.sqrt(v + eps)

def _scatter_add(tgt, idx, src, axis=0):
    return tgt.at[idx].add(src)

def _segment_sum(src, seg, n):
    return jax.ops.segment_sum(src, seg, n)

class _Rng:

    def __init__(self, key):
        self._k = key

    def _next(self):
        self._k, sub = jax.random.split(self._k)
        return sub

    def normal(self, shape):
        return jax.random.normal(self._next(), shape, dtype=jnp.bfloat16)

    def randint(self, lo, hi, shape):
        return jax.random.randint(self._next(), shape, lo, hi, dtype=jnp.int32)

    def uniform(self, shape, lo=0.0, hi=1.0):
        return jax.random.uniform(self._next(), shape, jnp.bfloat16, lo, hi)

    def permutation(self, n):
        return jax.random.permutation(self._next(), n)
kernel_name = 'recurrent_scan__memory_aug_recurrent_mem_tr__mixer_gmlp__prompt'

def setup_inputs():
    _rng = _Rng(jax.random.key(int.from_bytes(__import__("os").urandom(4), "little")))
    _w = lambda a: (lambda t: t.astype(jnp.bfloat16) if jnp.issubdtype(t.dtype, jnp.floating) else t)(jnp.asarray(a))

    def _A_setup():
        B, S, Dm = (1, 2048, 640)
        H, Dh = (32, 128)
        M, seg = (8, 32)
        seg = min(seg, S)
        S = S // seg * seg
        return {'x': _w((lambda *s: _rng.normal(s) * 0.05)(B, S, Dm)), 'mem0': _w((lambda *s: _rng.normal(s) * 0.1)(B, M, Dm)), 'Wq': _w((lambda *s: _rng.normal(s) * 1.6)(Dm, H, Dh) * Dm ** (-0.5)), 'Wk': _w((lambda *s: _rng.normal(s) * 1.6)(Dm, H, Dh) * Dm ** (-0.5)), 'Wv': _w((lambda *s: _rng.normal(s) * 0.1)(Dm, H, Dh) * Dm ** (-0.5)), 'Wo': _w((lambda *s: _rng.normal(s) * 0.1)(H, Dh, Dm) * (H * Dh) ** (-0.5)), 'seg_len': seg}
    _A_in = _A_setup()

    def _B_setup():
        B, S, D, F = (1, 2048, 640, 1728)
        Fh = F // 2
        return {'x': _w((lambda *s: _rng.normal(s) * 0.05)(B, S, D)), 'w_in': _w((lambda *s: _rng.normal(s) * 0.8)(D, 2 * Fh)), 'w_sp': _w(0.01 * (lambda *s: _rng.normal(s) * 0.8)(S, S)), 'b_sp': _w(1.0 + 0.01 * (lambda *s: _rng.normal(s) * 0.05)(S)), 'w_out': _w((lambda *s: _rng.normal(s) * 0.05)(Fh, D))}
    _B_in = _B_setup()
    return {'A_x': _A_in['x'], 'A_mem0': _A_in['mem0'], 'A_Wq': _A_in['Wq'], 'A_Wk': _A_in['Wk'], 'A_Wv': _A_in['Wv'], 'A_Wo': _A_in['Wo'], 'A_seg_len': _A_in['seg_len'], 'B_x': _B_in['x'], 'B_w_in': _B_in['w_in'], 'B_w_sp': _B_in['w_sp'], 'B_b_sp': _B_in['b_sp'], 'B_w_out': _B_in['w_out']}

def reference(A_x, A_mem0, A_Wq, A_Wk, A_Wv, A_Wo, A_seg_len, B_x, B_w_in, B_w_sp, B_b_sp, B_w_out):

    def _A_ref(x, mem0, Wq, Wk, Wv, Wo, seg_len):
        B, S, Dm = x.shape
        H, Dh = (Wq.shape[1], Wq.shape[2])
        M = mem0.shape[1]
        scale = Dh ** (-0.5)
        n_seg = S // seg_len
        L = M + seg_len
        idx = jnp.arange(L)
        mask = (idx[:, None] < M) | (idx[:, None] >= idx[None, :])
        mem = mem0
        outs = []
        for s in range(n_seg):
            xs = x[:, s * seg_len:(s + 1) * seg_len, :].copy()
            h = jnp.concatenate([mem, xs], axis=1)
            q = jnp.einsum('btd,dhe->bhte', h, Wq)
            k = jnp.einsum('btd,dhe->bhte', h, Wk)
            v = jnp.einsum('btd,dhe->bhte', h, Wv)
            scores = jnp.einsum('bhqe,bhke->bhqk', q, k) * scale
            scores = jnp.where(mask[None, None], scores, -1000000000.0)
            p = _softmax(scores, axis=-1)
            o = jnp.einsum('bhqk,bhke->bhqe', p, v)
            o = jnp.einsum('bhte,hed->btd', o, Wo)
            mem = o[:, :M, :].copy()
            outs.append(o[:, M:, :])
        return jnp.concatenate(outs, axis=1)

    def _B_ref(x, w_in, w_sp, b_sp, w_out):
        B, S, D = x.shape
        F = w_in.shape[-1]
        Fh = F // 2
        z = _gelu(jnp.einsum('bsd,df->bsf', x, w_in))
        z1 = z[..., :Fh].copy()
        z2 = _layernorm(z[..., Fh:], axis=-1)
        g = jnp.einsum('ts,bsf->btf', w_sp, z2) + b_sp[None, :, None]
        return jnp.einsum('bsf,fd->bsd', z1 * g, w_out)
    x = A_x
    xn = _layernorm(x, axis=-1)
    s = _A_ref(xn, A_mem0, A_Wq, A_Wk, A_Wv, A_Wo, A_seg_len)
    g = _silu(_B_ref(xn, B_w_in, B_w_sp, B_b_sp, B_w_out))
    return x + s * g
```

```python
import functools

import jax
import jax.numpy as jnp
import jax.experimental.pallas as pl
import jax.experimental.pallas.tpu as pltpu

F32 = jnp.float32
BF16 = jnp.bfloat16
U32 = jnp.uint32

LANES = 128
LN_EPS = 1e-5
LOG2E = 1.4426950408889634
MASK_VALUE = -1000000000.0
GELU_C1 = 0.7978845608028654
GELU_C2 = 0.044715 * GELU_C1

NN = (((1,), (0,)), ((), ()))
NT = (((1,), (1,)), ((), ()))

BM1 = 256
BM2 = 256
UNROLL = 2


def _dot(a, b, dims=NN):
    return jax.lax.dot_general(a, b, dims, preferred_element_type=F32)


def _gelu(x):
    t = jnp.tanh(x * (GELU_C1 + GELU_C2 * (x * x)))
    hx = 0.5 * x
    return hx + hx * t


def _head_schedule(heads, lag_scores=1, lag_pv=3, fill=(3, 5, 5)):
    ops = []
    for t in range(heads):
        ops.append(("qkv", t))
        if t >= lag_scores:
            ops.append(("scores", t - lag_scores))
        if t >= lag_pv:
            ops.append(("pv", t - lag_pv))
    nxt = 0
    for k, t in enumerate(range(heads, heads + lag_pv)):
        for _ in range(fill[min(k, len(fill) - 1)]):
            if nxt < t - lag_pv:
                ops.append(("out", nxt))
                nxt += 1
        if 0 <= t - lag_scores < heads:
            ops.append(("scores", t - lag_scores))
        if t >= lag_pv:
            ops.append(("pv", t - lag_pv))
    ops.extend(("out", h) for h in range(nxt, heads))
    return ops


def _kernel(
    x_hbm, mem_hbm, wq_hbm, wk_hbm, wv_hbm, wo_hbm, win_hbm, wsp_hbm, bsp_hbm, wout_hbm,
    out_hbm,
    x_v, mem_v, bsp_v, win_v, win2_v, wsp_v, wout_v, wstage_v, wqkv_v, wo_v,
    xn_v, bias_v, z1_v, z2_v, out_v,
    sem_x, sem_small, sem_win, sem_wsp, sem_w, sem_wo, sem_wout, sem_out,
    *, seq, dm, heads, dh, mem_rows, seg, fh,
):
    nd = dm // LANES
    nf = pl.cdiv(fh, LANES)
    f_tail = fh - (nf - 1) * LANES
    n1 = seq // BM1
    n2 = seq // BM2
    pairs = heads // 2
    pitch = dm // 2 + 8
    d_chunk = dm // n2

    def x_copy(i):
        rows = pl.ds(pl.multiple_of(i * BM1, BM1), BM1)
        return pltpu.make_async_copy(x_hbm.at[rows], x_v.at[rows], sem_x.at[i])

    def wsp_copy(i):
        rows = pl.ds(pl.multiple_of(i * BM2, BM2), BM2)
        return pltpu.make_async_copy(wsp_hbm.at[rows], wsp_v.at[rows], sem_wsp.at[i])

    def w_copy(j, i):
        n = d_chunk * heads
        rows = pl.ds(pl.multiple_of(i * n, n), n)
        src = (wq_hbm, wk_hbm, wv_hbm)[j]
        return pltpu.make_async_copy(src.at[rows], wstage_v.at[j, rows], sem_w.at[j, i])

    def wo_copy(n):
        cols = pl.ds(n * LANES, LANES)
        return pltpu.make_async_copy(wo_hbm.at[:, cols], wo_v.at[n], sem_wo.at[n])

    def wout_copy(n):
        cols = pl.ds(n * LANES, LANES)
        return pltpu.make_async_copy(
            wout_hbm.at[:, cols], wout_v.at[n, pl.ds(0, fh)], sem_wout.at[n])

    mem_copy = pltpu.make_async_copy(mem_hbm, mem_v, sem_small.at[0])
    bsp_copy = pltpu.make_async_copy(bsp_hbm, bsp_v, sem_small.at[1])
    win_copy = pltpu.make_async_copy(win_hbm, win_v, sem_win.at[0])

    x_copy(0).start()
    win_copy.start()
    bsp_copy.start()
    mem_copy.start()
    for i in range(1, n1):
        x_copy(i).start()

    def layernorm_x(i):
        rows = pl.ds(pl.multiple_of(i * BM1, BM1), BM1)
        x = x_v[rows, :].astype(F32)
        d = x - jnp.sum(x, axis=1, keepdims=True) * (1.0 / dm)
        var = jnp.sum(d * d, axis=1, keepdims=True) * (1.0 / dm)
        xn_v[rows, :] = d * jax.lax.rsqrt(var + LN_EPS)

    if nf * LANES > fh:
        wout_v[:, pl.ds(fh, nf * LANES - fh), :] = jnp.zeros((nd, nf * LANES - fh, LANES), BF16)

    x_copy(0).wait()
    layernorm_x(0)

    bsp_copy.wait()
    b = bsp_v[...].astype(F32)
    for j in range(seq // LANES):
        bias_v[pl.ds(j * LANES, LANES), :] = jnp.broadcast_to(b[j:j + 1, :], (LANES, LANES)).T

    win_copy.wait()
    for i in range(n2):
        wsp_copy(i).start()
        for j in range(3):
            w_copy(j, i).start()
    for n in range(nd):
        wout_copy(n).start()
    for n in range(nd):
        wo_copy(n).start()
    for n in range(nf):
        width = LANES if n < nf - 1 else f_tail
        w = win_v[:, pl.ds(fh + n * LANES, width)]
        if width < LANES:
            w = jnp.concatenate([w, jnp.zeros((dm, LANES - width), BF16)], axis=1)
        win2_v[n] = pltpu.bitcast(w, U32)

    tail_mask = jax.lax.broadcasted_iota(jnp.int32, (BM1, LANES), 1) < f_tail

    def project_in(i):
        rows = pl.ds(pl.multiple_of(i * BM1, BM1), BM1)
        xn = xn_v[rows, :]
        z2 = [_gelu(_dot(xn, pltpu.bitcast(win2_v[n], BF16))) for n in range(nf)]
        total = functools.reduce(lambda a, c: a + c, z2)
        mean = jnp.sum(total, axis=1, keepdims=True) * (1.0 / fh)
        d = [z - mean for z in z2]
        d[-1] = jnp.where(tail_mask, d[-1], 0.0)
        sq = functools.reduce(lambda a, c: a + c, [v * v for v in d])
        var = jnp.sum(sq, axis=1, keepdims=True) * (1.0 / fh)
        rstd = jax.lax.rsqrt(var + LN_EPS)
        half = pl.ds(pl.multiple_of(i * (BM1 // 2), BM1 // 2), BM1 // 2)
        for n in range(nf):
            z2_v[n, half, :] = pltpu.bitcast((d[n] * rstd).astype(BF16), U32)
        for n in range(nf):
            cols = pl.ds(n * LANES, LANES)
            z1 = _gelu(_dot(xn, win_v[:, cols]))
            if n == nf - 1:
                z1 = jnp.where(tail_mask, z1, 0.0)
            z1_v[rows, cols] = z1

    def phase1(i, carry):
        x_copy(i + 1).wait()
        layernorm_x(i + 1)
        project_in(i)
        return carry

    jax.lax.fori_loop(0, n1 - 1, phase1, 0)
    project_in(n1 - 1)

    stage32 = wstage_v.bitcast(U32)

    def relayout_weights(i):
        for j in range(3):
            for u in range(d_chunk // 2):
                d2 = i * (d_chunk // 2) + u
                for g in range(pairs // 8):
                    src = pl.multiple_of(d2 * 2 * pairs + g * 8, 8)
                    a = stage32[j, pl.ds(src, 8), :]
                    c = stage32[j, pl.ds(src + pairs, 8), :]
                    even = (a & jnp.uint32(0xFFFF)) | (c << 16)
                    odd = (a >> 16) | (c & jnp.uint32(0xFFFF0000))
                    base = (j * heads + g * 8) * pitch + d2
                    wqkv_v[pl.ds(base, 8, stride=pitch), :] = even
                    wqkv_v[pl.ds(base + pairs * pitch, 8, stride=pitch), :] = odd

    def phase2(i, carry):
        wsp_copy(i).wait()
        for j in range(3):
            w_copy(j, i).wait()
        rows = pl.ds(pl.multiple_of(i * BM2, BM2), BM2)
        w = wsp_v[rows, :]
        bias = bias_v[rows, :]
        for n in range(nf):
            cols = pl.ds(n * LANES, LANES)
            gate = _dot(w, pltpu.bitcast(z2_v[n], BF16)) + bias
            z1_v[rows, cols] = z1_v[rows, cols] * gate
        relayout_weights(i)
        return carry

    jax.lax.fori_loop(0, n2, phase2, 0)

    mem_copy.wait()
    for n in range(nd):
        wout_copy(n).wait()
    for n in range(nd):
        wo_copy(n).wait()

    rows_all = mem_rows + seg
    scale = dh ** -0.5
    qi = jax.lax.broadcasted_iota(jnp.int32, (rows_all, rows_all), 0)
    ki = jax.lax.broadcasted_iota(jnp.int32, (rows_all, rows_all), 1)
    mask = (qi < mem_rows) | (qi >= ki)
    schedule = _head_schedule(heads)
    wo32 = wo_v.bitcast(U32)
    wout32 = wout_v.bitcast(U32)

    def head_weights(h):
        slot = (h % 2) * pairs + h // 2
        return jnp.concatenate(
            [pltpu.bitcast(wqkv_v[pl.ds((j * heads + slot) * pitch, dm // 2), :], BF16)
             for j in range(3)], axis=1)

    def out_weights(h):
        rows = pl.ds(h * (dh // 2), dh // 2)
        return jnp.concatenate(
            [pltpu.bitcast(wo32[n, rows, :], BF16) for n in range(nd)], axis=1)

    def segment(s, mem):
        rows = pl.ds(pl.multiple_of(s * seg, seg), seg)
        hid = jnp.concatenate([mem, xn_v[rows, :]], axis=0)
        acc = None
        live = {}
        for op, h in schedule:
            if op == "qkv":
                r = _dot(hid, head_weights(h))
                live[h] = (r[:, :dh], r[:, dh:2 * dh], r[:, 2 * dh:])
            elif op == "scores":
                q, k, v = live[h]
                live[h] = (_dot(q, k.astype(BF16), NT), v)
            elif op == "pv":
                sc, v = live[h]
                sc = jnp.where(mask, sc, MASK_VALUE / scale)
                p = jnp.exp2((sc - jnp.max(sc, axis=1, keepdims=True)) * (scale * LOG2E))
                total = jnp.sum(p, axis=1, keepdims=True)
                live[h] = _dot(p, v.astype(BF16)) * (1.0 / total)
            else:
                y = _dot(live.pop(h), out_weights(h))
                acc = y if acc is None else acc + y
        return acc[:mem_rows], acc[mem_rows:]

    block = UNROLL * seg

    def out_copy(i):
        rows = pl.ds(pl.multiple_of(i * block, block), block)
        return pltpu.make_async_copy(out_v.at[rows], out_hbm.at[rows], sem_out.at[0])

    def phase3(i, mem):
        @pl.when(i > 0)
        def _():
            out_copy(i - 1).start()

        gate = None
        for u in range(UNROLL):
            s = i * UNROLL + u
            mem, attn = segment(s, mem)
            if u == 0:
                rows = pl.ds(pl.multiple_of(i * block, block), block)
                w = jnp.concatenate(
                    [pltpu.bitcast(wout32[n], BF16) for n in range(nd)], axis=1)
                y = _dot(z1_v[rows, :], w)
                gate = y * jax.nn.sigmoid(y)
            rows = pl.ds(pl.multiple_of(s * seg, seg), seg)
            res = x_v[rows, :].astype(F32) + attn * gate[u * seg:(u + 1) * seg]
            out_v[rows, :] = res.astype(BF16)
        return mem

    n3 = seq // block
    jax.lax.fori_loop(0, n3, phase3, mem_v[...].astype(F32))
    out_copy(n3 - 1).start()
    pltpu.make_async_copy(out_v, out_hbm, sem_out.at[0]).wait()


@functools.partial(jax.jit, static_argnames=("A_seg_len",))
def pallas_recurrent_scan__memory_aug_recurrent_mem_tr__mixer_gmlp__prompt_kernel(
    A_x: jax.Array,
    A_mem0: jax.Array,
    A_Wq: jax.Array,
    A_Wk: jax.Array,
    A_Wv: jax.Array,
    A_Wo: jax.Array,
    A_seg_len: int,
    B_x: jax.Array,
    B_w_in: jax.Array,
    B_w_sp: jax.Array,
    B_b_sp: jax.Array,
    B_w_out: jax.Array,
):
    del B_x
    batch, seq, dm = A_x.shape
    heads, dh = A_Wq.shape[1], A_Wq.shape[2]
    mem_rows = A_mem0.shape[1]
    seg = A_seg_len
    fh = B_w_in.shape[1] // 2
    assert batch == 1 and dh == LANES and dm % LANES == 0 and heads % 16 == 0
    assert seq % BM1 == 0 and seq % BM2 == 0 and seq % (UNROLL * seg) == 0
    assert mem_rows % 8 == 0 and seg % 16 == 0 and fh % 16 == 0
    assert dm % (2 * (seq // BM2)) == 0
    nd = dm // LANES
    nf = pl.cdiv(fh, LANES)
    pitch = dm // 2 + 8

    kernel = functools.partial(
        _kernel, seq=seq, dm=dm, heads=heads, dh=dh, mem_rows=mem_rows, seg=seg, fh=fh)
    hbm = pl.BlockSpec(memory_space=pltpu.MemorySpace.HBM)
    dma = pltpu.SemaphoreType.DMA
    out = pl.pallas_call(
        kernel,
        out_shape=jax.ShapeDtypeStruct((seq, dm), BF16),
        in_specs=[hbm] * 10,
        out_specs=hbm,
        scratch_shapes=[
            pltpu.VMEM((seq, dm), BF16),
            pltpu.VMEM((mem_rows, dm), BF16),
            pltpu.VMEM((seq // LANES, LANES), BF16),
            pltpu.VMEM((dm, 2 * fh), BF16),
            pltpu.VMEM((nf, dm // 2, LANES), U32),
            pltpu.VMEM((seq, seq), BF16),
            pltpu.VMEM((nd, nf * LANES, LANES), BF16),
            pltpu.VMEM((3, dm * heads, dh), BF16),
            pltpu.VMEM((3 * heads * pitch, dh), U32),
            pltpu.VMEM((nd, heads * dh, LANES), BF16),
            pltpu.VMEM((seq, dm), F32),
            pltpu.VMEM((seq, LANES), F32),
            pltpu.VMEM((seq, nf * LANES), F32),
            pltpu.VMEM((nf, seq // 2, LANES), U32),
            pltpu.VMEM((seq, dm), BF16),
            dma((seq // BM1,)), dma((2,)), dma((1,)), dma((seq // BM2,)),
            dma((3, seq // BM2)), dma((nd,)), dma((nd,)), dma((1,)),
        ],
        compiler_params=pltpu.CompilerParams(vmem_limit_bytes=100 * 1024 * 1024),
    )(
        A_x.reshape(seq, dm),
        A_mem0.reshape(mem_rows, dm),
        A_Wq.reshape(dm * heads, dh),
        A_Wk.reshape(dm * heads, dh),
        A_Wv.reshape(dm * heads, dh),
        A_Wo.reshape(heads * dh, dm),
        B_w_in,
        B_w_sp,
        B_b_sp.reshape(seq // LANES, LANES),
        B_w_out,
    )
    return out.reshape(batch, seq, dm).astype(A_x.dtype)
```

```python
import functools

import jax
import jax.numpy as jnp
import jax.experimental.pallas as pl
import jax.experimental.pallas.tpu as pltpu

F32 = jnp.float32
BF16 = jnp.bfloat16
U32 = jnp.uint32

LANES = 128
LN_EPS = 1e-5
LOG2E = 1.4426950408889634
MASK_VALUE = -1000000000.0
GELU_C1 = 0.7978845608028654
GELU_C2 = 0.044715 * GELU_C1

NN = (((1,), (0,)), ((), ()))
NT = (((1,), (1,)), ((), ()))

BT1 = 256
BT2 = 512
LN_ROWS = 32
FC1 = 96
BT1B = 512
LEVELS = 2
PREP_ROWS = 8
FC2 = 216
FLAGS = None
SLOTS = (1, 1, 1, 1)
RELAYOUT_ROWS = 32
KV_DTYPE = BF16
SCHED = (2, 5, (4,), 28)
UNROLL = 4


def _dot(a, b, dims=NN):
    return jax.lax.dot_general(a, b, dims, preferred_element_type=F32)


def _gelu(x):
    t = jnp.tanh(x * (GELU_C1 + GELU_C2 * (x * x)))
    hx = 0.5 * x
    return hx + hx * t


def _chunks(total, size):
    return [(lo, min(size, total - lo)) for lo in range(0, total, size)]


def _fold_rows(x):
    return functools.reduce(lambda a, b: a + b, [x[r:r + 8] for r in range(0, x.shape[0], 8)])


def _tile_rows(x, rows):
    return jnp.concatenate([x] * (rows // x.shape[0]), axis=0)


def _interleave(main, side):
    done = 0
    for k, fn in enumerate(main):
        fn()
        upto = len(side) * (k + 1) // len(main)
        for g in side[done:upto]:
            g()
        done = upto
    for g in side[done:]:
        g()


def _start(copies):
    for cp in copies:
        cp.start()


def _wait(copies):
    for cp in copies:
        cp.wait()


STRASSEN_LHS = (
    ((0, 0, 1), (1, 1, 1)), ((1, 0, 1), (1, 1, 1)), ((0, 0, 1),), ((1, 1, 1),),
    ((0, 0, 1), (0, 1, 1)), ((1, 0, 1), (0, 0, -1)), ((0, 1, 1), (1, 1, -1)))
STRASSEN_RHS = (
    ((0, 0, 1), (1, 1, 1)), ((0, 0, 1),), ((0, 1, 1), (1, 1, -1)), ((1, 0, 1), (0, 0, -1)),
    ((1, 1, 1),), ((0, 0, 1), (0, 1, 1)), ((1, 0, 1), (1, 1, 1)))
STRASSEN_OUT = (
    (((0, 1), (3, 1), (4, -1), (6, 1)), ((2, 1), (4, 1))),
    (((1, 1), (3, 1)), ((0, 1), (1, -1), (2, 1), (5, 1))))
STRASSEN_ORDER = (4, 1, 0, 3, 6, 2, 5)


def _signed_sum(terms):
    total = terms[0][0]
    for value, sign in terms[1:]:
        total, value = total.astype(F32), value.astype(F32)
        total = total + value if sign > 0 else total - value
    return total


def _strassen_factor(terms, grid):
    half = len(grid) // 2
    return [
        [_signed_sum([(grid[r * half + a][c * half + b], sign) for r, c, sign in terms])
         for b in range(half)] for a in range(half)]


def _strassen_left_factors(grid):
    if len(grid) == 1:
        return [grid[0][0]]
    return sum((_strassen_left_factors(_strassen_factor(t, grid)) for t in STRASSEN_LHS), [])


def _strassen_multiply(product, right, finished=None, index=0):
    half = len(right) // 2
    if not half:
        return [[product(index, right[0][0])]]
    grid = [[None] * (2 * half) for _ in range(2 * half)]
    for k, m in enumerate(STRASSEN_ORDER):
        inner = _strassen_multiply(
            product, _strassen_factor(STRASSEN_RHS[m], right), None, index * 7 + m)
        for r in range(2):
            for c in range(2):
                for sign in [sign for q, sign in STRASSEN_OUT[r][c] if q == m]:
                    cells = [(r * half + a, c * half + b, inner[a][b])
                             for a in range(half) for b in range(half)]
                    for row, col, new in cells:
                        old = grid[row][col]
                        if old is None:
                            grid[row][col] = new if sign > 0 else -new
                        else:
                            grid[row][col] = old + new if sign > 0 else old - new
                    done = all(q in STRASSEN_ORDER[:k + 1] for q, _ in STRASSEN_OUT[r][c])
                    if finished and done:
                        finished([(row, col, grid[row][col]) for row, col, _ in cells])
    return grid


def _head_schedule(heads, lag_scores, lag_pv, fill, lag_out=None):
    ops = []
    nxt = 0
    for t in range(heads + lag_pv):
        if t < heads:
            ops.append(("qkv", t))
            count = int(lag_out is not None and t >= lag_out)
        else:
            count = fill[min(t - heads, len(fill) - 1)]
        for _ in range(count):
            if nxt < t - lag_pv:
                ops.append(("out", nxt))
                nxt += 1
        if 0 <= t - lag_scores < heads:
            ops.append(("scores", t - lag_scores))
        if t >= lag_pv:
            ops.append(("pv", t - lag_pv))
    ops.extend(("out", h) for h in range(nxt, heads))
    return ops


def _kernel(
    x_hbm, mem_hbm, wq_hbm, wk_hbm, wv_hbm, wo_hbm, win_hbm, wsp_hbm, bsp_hbm, wout_hbm,
    out_hbm,
    x_v, mem_v, bsp_v, win_v, wsp_v, wout_v, wstage_v, words_v, wo_v,
    xn_v, stat_v, z2t_v, mix_v, out_v,
    sem_x, sem_small, sem_win, sem_w, sem_wo, sem_out,
    *, seq, dm, heads, dh, mem_rows, seg, fh,
):
    nd = dm // LANES
    nf = pl.cdiv(fh, LANES)
    n1 = seq // BT1
    n2 = seq // BT2
    pairs = heads // 2
    pair_chunk = pairs // n2

    def x_copy(i):
        rows = pl.ds(pl.multiple_of(i * BT1, BT1), BT1)
        return pltpu.make_async_copy(x_hbm.at[rows], x_v.at[rows], sem_x.at[i])

    def win_copies(part):
        rows = pl.ds(part * fh, fh)
        return [
            pltpu.make_async_copy(
                win_hbm.at[rows, pl.ds(k * LANES, LANES)], win_v.at[k, rows], sem_win.at[part])
            for k in range(nd)
        ]

    def phase2_copies(i):
        rows = pl.ds(pl.multiple_of(i * BT2, BT2), BT2)
        return [
            pltpu.make_async_copy(
                wsp_hbm.at[rows, pl.ds(k * LANES, LANES)], wsp_v.at[k, rows], sem_w.at[i])
            for k in range(seq // LANES)
        ] + [
            pltpu.make_async_copy(
                src.bitcast(U32).at[:, odd, i * pair_chunk + g],
                wstage_v.at[j, i * pair_chunk + g, odd], sem_w.at[i])
            for j, src in enumerate((wq_hbm, wk_hbm, wv_hbm))
            for g in range(pair_chunk) for odd in range(2)
        ]

    phase3_copies = [
        pltpu.make_async_copy(
            wout_hbm.at[:, pl.ds(n * LANES, LANES)], wout_v.at[n, pl.ds(0, fh)], sem_wo.at[0])
        for n in range(nd)
    ] + [
        pltpu.make_async_copy(wo_hbm.at[:, pl.ds(n * LANES, LANES)], wo_v.at[n], sem_wo.at[0])
        for n in range(nd)
    ]
    mem_copy = pltpu.make_async_copy(mem_hbm, mem_v, sem_small.at[0])
    bsp_copy = pltpu.make_async_copy(bsp_hbm, bsp_v, sem_small.at[1])

    x_copy(0).start()
    x_copy(1).start()
    _start(win_copies(1))

    if nf * LANES > fh:
        wout_v[:, pl.ds(fh, nf * LANES - fh), :] = jnp.zeros((nd, nf * LANES - fh, LANES), BF16)

    def layernorm_x(i):
        def piece(r):
            rows = pl.ds(pl.multiple_of(i * BT1 + r, LN_ROWS), LN_ROWS)
            x = x_v[rows, :].astype(F32)
            d = x - jnp.sum(x, axis=1, keepdims=True) * (1.0 / dm)
            var = jnp.sum(d * d, axis=1, keepdims=True) * (1.0 / dm)
            xn_v[rows, :] = d * jax.lax.rsqrt(var + LN_EPS)

        return [functools.partial(piece, r) for r in range(0, BT1, LN_ROWS)]

    win32 = win_v.bitcast(U32)

    def load_win(lo, size):
        rows = pl.ds(lo // 2, size // 2)
        return jnp.concatenate([pltpu.bitcast(win32[k, rows, :], BF16) for k in range(nd)], axis=1)

    def load_xn(first, count):
        return xn_v[pl.ds(pl.multiple_of(first, count), count), :]

    def project_in(half, tile, store):
        xn = load_xn(tile * LANES, LANES).astype(BF16)

        def piece(lo, size):
            store(tile, lo, size, _gelu(_dot(load_win(half * fh + lo, size), xn, NT)))

        return [functools.partial(piece, lo, size) for lo, size in _chunks(fh, FC1)]

    def gate_half(tile):
        acc = {}

        def store(tile, lo, size, z):
            if lo == 0:
                acc["pilot"] = jnp.sum(_fold_rows(z), axis=0, keepdims=True) * (1.0 / size)
                acc["s1"] = acc["s2"] = 0.0
            d = z - acc["pilot"]
            z2t_v[tile, pl.ds(lo, size), :] = d
            acc["s1"] += _fold_rows(d)
            acc["s2"] += _fold_rows(d * d)
            if lo + size == fh:
                stat_v[tile, 0] = acc["s1"]
                stat_v[tile, 1] = acc["s2"]

        return project_in(1, tile, store)

    early = n2 // 2

    def phase1(i, carry):
        @pl.when(i + 1 < n1)
        def _():
            x_copy(i + 1).wait()

        tiles = BT1 // LANES
        _interleave(
            sum((gate_half(i * tiles + u) for u in range(tiles)), []),
            layernorm_x(jnp.minimum(i + 1, n1 - 1)))

        return carry

    with jax.named_scope("wait_x0"):
        x_copy(0).wait()
    for i in range(2, n1):
        x_copy(i).start()
    with jax.named_scope("ln0"):
        _interleave(layernorm_x(0), [])
    with jax.named_scope("wait_win"):
        _wait(win_copies(1))
    _start(win_copies(0))
    bsp_copy.start()
    mem_copy.start()
    for c in range(early // 2):
        _start(phase2_copies(c))
    with jax.named_scope("phase1"):
        jax.lax.fori_loop(0, n1, phase1, 0)

    side = 2 ** LEVELS
    fs = fh // side
    groups = seq // LANES // side
    products = 7 ** LEVELS

    def z1_rows(tile, lo, size):
        return pl.ds(pl.multiple_of(tile * fh + lo, 8), size)

    def lhs_rows(product, group, lo, size):
        first = seq // LANES * fh + (product * groups + group) * fs + lo
        return pl.ds(pl.multiple_of(first, 8), size)

    def store_z1(tile, lo, size, z):
        mix_v[z1_rows(tile, lo, size), :] = z

    def left_factors(group):
        def piece(lo, size):
            grid = [
                [(z2t_v[group * side + k, pl.ds(r * fs + lo, size), :]
                  - _tile_rows(stat_v[group * side + k, 0], size))
                 * _tile_rows(stat_v[group * side + k, 1], size)
                 for k in range(side)] for r in range(side)]
            for m, factor in enumerate(_strassen_left_factors(grid)):
                mix_v[lhs_rows(m, group, lo, size), :] = factor

        return [functools.partial(piece, lo, size) for lo, size in _chunks(fs, PREP_ROWS)]

    def phase1b(i, carry):
        tiles = BT1B // LANES
        _interleave(
            sum((project_in(0, i * tiles + u, store_z1) for u in range(tiles)), []),
            sum((left_factors(i * (tiles // side) + g) for g in range(tiles // side)), []))

        @pl.when(i == 0)
        def _():
            for c in range(early // 2, early):
                _start(phase2_copies(c))

        return carry

    for tile in range(seq // LANES):
        shift = jnp.sum(stat_v[tile, 0], axis=0, keepdims=True) * (1.0 / fh)
        var = jnp.sum(stat_v[tile, 1], axis=0, keepdims=True) * (1.0 / fh) - shift * shift
        rstd = jax.lax.rsqrt(jnp.maximum(var, 0.0) + LN_EPS)
        stat_v[tile, 0] = jnp.broadcast_to(shift, (8, LANES))
        stat_v[tile, 1] = jnp.broadcast_to(rstd, (8, LANES))
    with jax.named_scope("wait_win0"):
        _wait(win_copies(0))
        bsp_copy.wait()
    with jax.named_scope("phase1b"):
        jax.lax.fori_loop(0, seq // BT1B, phase1b, 0)

    def w_rows(head, j, lo, size):
        return pl.ds(pl.multiple_of((head * 3 + j) * (dm // 2) + lo, 8), size)

    def zg_rows(tile, lo, size):
        return pl.ds(pl.multiple_of(heads * 3 * (dm // 2) + tile * fh + lo, 8), size)

    def relayout_weights(i, part):
        work = [(j, g, r) for j in range(3) for g in range(pair_chunk)
                for r in range(0, dm // 2, RELAYOUT_ROWS)]
        first, last = (len(work) * sum(SLOTS[:k]) // sum(SLOTS) for k in (part, part + 1))
        for j, g, r in work[first:last]:
            pair = i * pair_chunk + g
            a = wstage_v[j, pair, 0, pl.ds(r, RELAYOUT_ROWS), :]
            c = wstage_v[j, pair, 1, pl.ds(r, RELAYOUT_ROWS), :]
            words_v[w_rows(2 * pair, j, r, RELAYOUT_ROWS), :] = (
                (a & jnp.uint32(0xFFFF)) | (c << 16))
            words_v[w_rows(2 * pair + 1, j, r, RELAYOUT_ROWS), :] = (
                (a >> 16) | (c & jnp.uint32(0xFFFF0000)))

    chunks2 = _chunks(fs, FC2)
    wsp32 = wsp_v.bitcast(U32)

    def mixing_blocks(group):
        def tile(source, target):
            rows = pl.ds(pl.multiple_of(target * (LANES // 2), LANES // 2), LANES // 2)
            return pltpu.bitcast(wsp32[source, rows, :], BF16)

        return [
            [jnp.concatenate(
                [tile(g * side + k, group * side + c) for g in range(groups)], axis=1)
             for c in range(side)] for k in range(side)]

    def bias_row(tile):
        bias = bsp_v[...].astype(F32)
        pick = jax.lax.broadcasted_iota(jnp.int32, bias.shape, 0) == tile
        return jnp.sum(jnp.where(pick, bias, 0.0), axis=0, keepdims=True)

    def phase2(i, carry):
        for c in range(n2 - early):
            pl.when(i == c)(lambda: _start(phase2_copies(c + early)))
        pl.when(i == n2 - early)(lambda: _start(phase3_copies))
        _wait(phase2_copies(i))
        count = BT2 // LANES // side
        reported = []
        relayout_weights(i, 0)
        for u in range(count):
            group = i * count + u
            bias = [bias_row(group * side + c) for c in range(side)]
            for n, (lo, size) in enumerate(chunks2):
                def product(m, rhs):
                    lhs = jnp.concatenate(
                        [mix_v[lhs_rows(m, g, lo, size), :] for g in range(groups)], axis=1)
                    return _dot(lhs, rhs.astype(BF16), NT)

                def finished(blocks):
                    for r, c, gate in blocks:
                        at = (group * side + c, r * fs + lo, size)
                        zg = mix_v[z1_rows(*at), :] * (gate + bias[c])
                        words_v[zg_rows(*at), :] = pltpu.bitcast(zg, U32)
                    reported.append(None)
                    relayout_weights(i, len(reported))

                _strassen_multiply(product, mixing_blocks(group), finished)
        return carry

    with jax.named_scope("phase2"):
        jax.lax.fori_loop(0, n2, phase2, 0)

    with jax.named_scope("wait_wo"):
        mem_copy.wait()
        _wait(phase3_copies)

    rows_all = mem_rows + seg
    scale = dh ** -0.5
    qi = jax.lax.broadcasted_iota(jnp.int32, (rows_all, rows_all), 0)
    ki = jax.lax.broadcasted_iota(jnp.int32, (rows_all, rows_all), 1)
    mask = (qi < mem_rows) | (qi >= ki)
    schedule = _head_schedule(heads, *SCHED)
    wo32 = wo_v.bitcast(U32)
    wout32 = wout_v.bitcast(U32)

    def head_weights(h):
        return jnp.concatenate(
            [pltpu.bitcast(words_v[pl.ds((h * 3 + j) * (dm // 2), dm // 2), :], BF16)
             for j in range(3)], axis=1)

    def out_weights(h):
        rows = pl.ds(h * (dh // 2), dh // 2)
        return jnp.concatenate(
            [pltpu.bitcast(wo32[n, rows, :], BF16) for n in range(nd)], axis=1)

    def segment(s, mem):
        hid = jnp.concatenate([mem, load_xn(s * seg, seg)], axis=0)
        acc = None
        live = {}
        for op, h in schedule:
            if op == "qkv":
                r = _dot(hid, head_weights(h))
                live[h] = (r[:, :dh], r[:, dh:2 * dh], r[:, 2 * dh:])
            elif op == "scores":
                q, k, v = live[h]
                live[h] = (_dot(q, k.astype(KV_DTYPE), NT), v)
            elif op == "pv":
                sc, v = live[h]
                sc = jnp.where(mask, sc, MASK_VALUE / scale)
                p = jnp.exp2((sc - jnp.max(sc, axis=1, keepdims=True)) * (scale * LOG2E))
                total = jnp.sum(p, axis=1, keepdims=True)
                live[h] = _dot(p, v.astype(KV_DTYPE)) * (1.0 / total)
            else:
                y = _dot(live.pop(h), out_weights(h))
                acc = y if acc is None else acc + y
        return acc[:mem_rows], acc[mem_rows:]

    block = UNROLL * seg

    def out_copy(i):
        rows = pl.ds(pl.multiple_of(i * block, block), block)
        return pltpu.make_async_copy(out_v.at[rows], out_hbm.at[rows], sem_out.at[0])

    def phase3(i, mem):
        @pl.when(i > 0)
        def _():
            out_copy(i - 1).start()

        zg = []
        for lo, size in _chunks(fh, LANES):
            t = pltpu.bitcast(words_v[zg_rows(i, lo, size), :], F32)
            if size < LANES:
                t = jnp.concatenate([t, jnp.zeros((LANES - size, LANES), F32)], axis=0)
            zg.append(t.T)
        zg = jnp.concatenate(zg, axis=1)

        def gate_rows(first, count):
            w = jnp.concatenate([pltpu.bitcast(wout32[n], BF16) for n in range(nd)], axis=1)
            y = _dot(zg[first * seg:(first + count) * seg], w)
            g = y * jax.nn.sigmoid(y)
            return [g[c * seg:(c + 1) * seg] for c in range(count)]

        gates = []
        for u in range(UNROLL):
            s = i * UNROLL + u
            mem, attn = segment(s, mem)
            if u < UNROLL - 2:
                gates += gate_rows(u, 1)
            elif u == UNROLL - 2:
                gates += gate_rows(u, 2)
            elif UNROLL == 1:
                gates += gate_rows(u, 1)
            rows = pl.ds(pl.multiple_of(s * seg, seg), seg)
            res = x_v[rows, :].astype(F32) + attn * gates[u]
            out_v[rows, :] = res.astype(BF16)
        return mem

    n3 = seq // block
    with jax.named_scope("phase3"):
        jax.lax.fori_loop(0, n3, phase3, mem_v[...].astype(F32))
    with jax.named_scope("wait_out"):
        out_copy(n3 - 1).start()
        pltpu.make_async_copy(out_v, out_hbm, sem_out.at[0]).wait()


@functools.partial(jax.jit, static_argnames=("A_seg_len",))
def pallas_recurrent_scan__memory_aug_recurrent_mem_tr__mixer_gmlp__prompt_kernel(
    A_x: jax.Array,
    A_mem0: jax.Array,
    A_Wq: jax.Array,
    A_Wk: jax.Array,
    A_Wv: jax.Array,
    A_Wo: jax.Array,
    A_seg_len: int,
    B_x: jax.Array,
    B_w_in: jax.Array,
    B_w_sp: jax.Array,
    B_b_sp: jax.Array,
    B_w_out: jax.Array,
):
    del B_x
    batch, seq, dm = A_x.shape
    heads, dh = A_Wq.shape[1], A_Wq.shape[2]
    mem_rows = A_mem0.shape[1]
    seg = A_seg_len
    fh = B_w_in.shape[1] // 2
    assert batch == 1 and dh == LANES and dm % LANES == 0
    assert seq % BT2 == 0 and seq % BT1 == 0 and UNROLL * seg == LANES
    assert mem_rows % 8 == 0 and seg % 16 == 0 and fh % 16 == 0
    assert heads % (2 * (seq // BT2)) == 0 and dm % (2 * RELAYOUT_ROWS) == 0
    nd = dm // LANES
    nf = pl.cdiv(fh, LANES)

    kernel = functools.partial(
        _kernel, seq=seq, dm=dm, heads=heads, dh=dh, mem_rows=mem_rows, seg=seg, fh=fh)
    hbm = pl.BlockSpec(memory_space=pltpu.MemorySpace.HBM)
    dma = pltpu.SemaphoreType.DMA
    out = pl.pallas_call(
        kernel,
        out_shape=jax.ShapeDtypeStruct((seq, dm), BF16),
        in_specs=[hbm] * 10,
        out_specs=hbm,
        scratch_shapes=[
            pltpu.VMEM((seq, dm), BF16),
            pltpu.VMEM((mem_rows, dm), BF16),
            pltpu.VMEM((seq // LANES, LANES), BF16),
            pltpu.VMEM((nd, 2 * fh, LANES), BF16),
            pltpu.VMEM((seq // LANES, seq, LANES), BF16),
            pltpu.VMEM((nd, nf * LANES, LANES), BF16),
            pltpu.VMEM((3, heads // 2, 2, dm // 2, dh), U32),
            pltpu.VMEM((heads * 3 * dm // 2 + seq // LANES * fh, LANES), U32),
            pltpu.VMEM((nd, heads * dh, LANES), BF16),
            pltpu.VMEM((seq, dm), F32),
            pltpu.VMEM((seq // LANES, 2, 8, LANES), F32),
            pltpu.VMEM((seq // LANES, fh, LANES), F32),
            pltpu.VMEM((seq // LANES * fh * (4 ** LEVELS + 7 ** LEVELS) // 4 ** LEVELS, LANES), F32),
            pltpu.VMEM((seq, dm), BF16),
            dma((seq // BT1,)), dma((2,)), dma((2,)), dma((seq // BT2,)),
            dma((1,)), dma((1,)),
        ],
        compiler_params=pltpu.CompilerParams(vmem_limit_bytes=116 * 1024 * 1024, flags=FLAGS),
    )(
        A_x.reshape(seq, dm),
        A_mem0.reshape(mem_rows, dm),
        A_Wq.reshape(dm // 2, 2, heads, dh),
        A_Wk.reshape(dm // 2, 2, heads, dh),
        A_Wv.reshape(dm // 2, 2, heads, dh),
        A_Wo.reshape(heads * dh, dm),
        B_w_in.T,
        B_w_sp,
        B_b_sp.reshape(seq // LANES, LANES),
        B_w_out,
    )
    return out.reshape(batch, seq, dm).astype(A_x.dtype)
```

```python
import functools
import itertools
import math

import jax
import jax.numpy as jnp
import jax.experimental.pallas as pl
import jax.experimental.pallas.tpu as pltpu

F32 = jnp.float32
BF16 = jnp.bfloat16
U32 = jnp.uint32

LANES = 128
LN_EPS = 1e-5
LOG2E = 1.4426950408889634
MASK_VALUE = -1000000000.0
GELU_C1 = 0.7978845608028654
GELU_C2 = 0.044715 * GELU_C1

NN = (((1,), (0,)), ((), ()))
NT = (((1,), (1,)), ((), ()))

STRASSEN_LHS = (
    ((0, 0, 1), (1, 1, 1)), ((1, 0, 1), (1, 1, 1)), ((0, 0, 1),), ((1, 1, 1),),
    ((0, 0, 1), (0, 1, 1)), ((1, 0, 1), (0, 0, -1)), ((0, 1, 1), (1, 1, -1)))
STRASSEN_RHS = (
    ((0, 0, 1), (1, 1, 1)), ((0, 0, 1),), ((0, 1, 1), (1, 1, -1)), ((1, 0, 1), (0, 0, -1)),
    ((1, 1, 1),), ((0, 0, 1), (0, 1, 1)), ((1, 0, 1), (1, 1, 1)))
STRASSEN_OUT = (
    (((0, 1), (3, 1), (4, -1), (6, 1)), ((2, 1), (4, 1))),
    (((1, 1), (3, 1)), ((0, 1), (1, -1), (2, 1), (5, 1))))
SIDE = 4
PRODUCTS = 49
BLOCK = SIDE * LANES

LN_ROWS = 32
IN_ROWS = (80, 96)
MIX_ORDER = ((4, 1, 3, 0, 6, 2, 5), (4, 1, 0, 3, 6, 2, 5))
AHEAD_ORDER = ((1, 4, 0, 5, 3, 6, 2), (4, 1, 0, 3, 6, 2, 5))
REST_AFTER = 7
RELAYOUT_AFTER = (2, 9, 16)
RELAYOUT_ROWS = 64
RINGS = 8
LAG_SCORES, LAG_PV = 3, 6
FIRST_OUT, OUT_PERIOD, LAST_OUTS = 17, 2, (2, 3, 3, 3, 4, 3)
GATE_ROWS = (0, 48, 80, LANES)


def _dot(a, b, dims=NN):
    return jax.lax.dot_general(a, b, dims, preferred_element_type=F32)


def _gelu(x):
    t = jnp.tanh(x * (GELU_C1 + GELU_C2 * (x * x)))
    hx = 0.5 * x
    return hx + hx * t


def _chunks(total, size):
    return [(lo, min(size, total - lo)) for lo in range(0, total, size)]


def _fold_rows(x):
    return functools.reduce(lambda a, b: a + b, [x[r:r + 8] for r in range(0, x.shape[0], 8)])


def _interleave(main, side):
    merged, done = [], 0
    for k, item in enumerate(main):
        upto = len(side) * (k + 1) // len(main)
        merged += [item] + side[done:upto]
        done = upto
    return merged


def _run(thunks):
    for fn in thunks:
        fn()


def _start(copies):
    for cp in copies:
        cp.start()


def _wait(copies):
    for cp in copies:
        cp.wait()


def _signed_sum(terms):
    total = terms[0][0]
    for value, sign in terms[1:]:
        total, value = total.astype(F32), value.astype(F32)
        total = total + value if sign > 0 else total - value
    return total


def _strassen_factor(terms, grid):
    half = len(grid) // 2
    return [
        [_signed_sum([(grid[r * half + a][c * half + b], sign) for r, c, sign in terms])
         for b in range(half)] for a in range(half)]


def _strassen_left_factors(grid):
    if len(grid) == 1:
        return [grid[0][0]]
    return sum((_strassen_left_factors(_strassen_factor(t, grid)) for t in STRASSEN_LHS), [])


def _strassen_multiply(order, product, right, finished=None, index=0):
    half = len(right) // 2
    if not half:
        return [[product(index, right[0][0])]]
    grid = [[None] * (2 * half) for _ in range(2 * half)]
    for k, m in enumerate(order[0]):
        inner = _strassen_multiply(
            order[1:], product, _strassen_factor(STRASSEN_RHS[m], right), None, index * 7 + m)
        for r, c in itertools.product(range(2), range(2)):
            for sign in [sign for q, sign in STRASSEN_OUT[r][c] if q == m]:
                cells = [(r * half + a, c * half + b, inner[a][b])
                         for a in range(half) for b in range(half)]
                for row, col, new in cells:
                    old = grid[row][col]
                    if old is None:
                        grid[row][col] = new if sign > 0 else -new
                    else:
                        grid[row][col] = old + new if sign > 0 else old - new
                if finished and all(q in order[0][:k + 1] for q, _ in STRASSEN_OUT[r][c]):
                    finished([(row, col, grid[row][col]) for row, col, _ in cells])
    return grid


def _head_schedule(heads):
    ops = []
    out = 0
    for t in range(heads + LAG_PV):
        if t < heads:
            count = int(t >= FIRST_OUT and (t - FIRST_OUT) % OUT_PERIOD == 0)
        else:
            count = LAST_OUTS[t - heads]
        for _ in range(count):
            if out < t - LAG_PV:
                ops.append(("out", out))
                out += 1
        if t < heads:
            ops.append(("qkv", t))
        if 0 <= t - LAG_SCORES < heads:
            ops.append(("scores", t - LAG_SCORES))
        if t >= LAG_PV:
            ops.append(("pv", t - LAG_PV))
    return ops + [("out", h) for h in range(out, heads)]


def _kernel(
    x_hbm, mem_hbm, wq_hbm, wk_hbm, wv_hbm, wo_hbm, win_hbm, wsp_hbm, bsp_hbm, wout_hbm,
    out_hbm,
    x_v, mem_v, wout_v, wo_v, words_v, mix_v, out_v,
    sem_x, sem_small, sem_win, sem_w, sem_wo, sem_out,
    *, seq, dm, heads, dh, mem_rows, seg, fh,
):
    nd = dm // LANES
    nf = pl.cdiv(fh, LANES)
    tiles = seq // LANES
    groups = seq // BLOCK
    fs = fh // SIDE
    pair_chunk = heads // 2 // groups
    ride = seg - BLOCK * seg // seq
    ring_rows = pl.cdiv(BLOCK + ride, math.lcm(seg, ride)) * math.lcm(seg, ride)

    def xn_rows(k, first, count):
        return pl.ds(pl.multiple_of(k * seq + first, 8), count)

    def z1_rows(tile, lo, size):
        return pl.ds(pl.multiple_of(nd * seq + tile * fh + lo, 8), size)

    def mixing_rows(product, group, lo, size):
        first = nd * seq + tiles * fh + (product * groups + group) * fs + lo
        return pl.ds(pl.multiple_of(first, 8), size)

    def ahead_rows(product, lo, size):
        return pl.ds(nd * seq + tiles * fh + PRODUCTS * groups * fs + product * LANES + lo, size)

    def w_rows(tile, lo, size):
        return pl.ds(pl.multiple_of(tile * (dm // 2) + lo, 8), size)

    def zg_rows(tile, lo, size):
        return pl.ds(pl.multiple_of(heads * 3 * (dm // 2) + tile * fh + lo, 8), size)

    def load_xn(first, count):
        return jnp.concatenate([mix_v[xn_rows(k, first, count), :] for k in range(nd)], axis=1)

    mem_copy = pltpu.make_async_copy(mem_hbm, mem_v, sem_small.at[0])
    late_copies = [
        pltpu.make_async_copy(
            wout_hbm.at[:, pl.ds(n * LANES, LANES)], wout_v.at[n, pl.ds(0, fh)], sem_wo.at[0])
        for n in range(nd)
    ] + [
        pltpu.make_async_copy(wo_hbm.at[:, pl.ds(n * LANES, LANES)], wo_v.at[n], sem_wo.at[0])
        for n in range(nd)
    ]

    def gmlp(bsp_v, win_v, wsp_v, wstage_v, stat_v, z2t_v):
        def x_copy(i):
            rows = pl.ds(pl.multiple_of(i * BLOCK, BLOCK), BLOCK)
            return pltpu.make_async_copy(x_hbm.at[rows], x_v.at[rows], sem_x.at[i])

        def win_copies(half):
            rows = pl.ds(half * fh, fh)
            return [
                pltpu.make_async_copy(
                    win_hbm.at[rows, pl.ds(k * LANES, LANES)], win_v.at[k, rows], sem_win.at[half])
                for k in range(nd)
            ]

        def phase2_copies(i):
            rows = pl.ds(pl.multiple_of(i * BLOCK, BLOCK), BLOCK)
            return [
                pltpu.make_async_copy(
                    wsp_hbm.at[rows, pl.ds(k * LANES, LANES)], wsp_v.at[k, rows], sem_w.at[i])
                for k in range(tiles)
            ] + [
                pltpu.make_async_copy(
                    src.bitcast(U32).at[:, odd, i * pair_chunk + g],
                    wstage_v.at[j, i * pair_chunk + g, odd], sem_w.at[i])
                for j, src in enumerate((wq_hbm, wk_hbm, wv_hbm))
                for g in range(pair_chunk) for odd in range(2)
            ]

        bsp_copy = pltpu.make_async_copy(bsp_hbm, bsp_v, sem_small.at[1])
        bsp_copy.start()
        x_copy(0).start()
        bsp_copy.wait()
        _start(win_copies(1))

        if nf * LANES > fh:
            wout_v[:, pl.ds(fh, nf * LANES - fh), :] = jnp.zeros(
                (nd, nf * LANES - fh, LANES), BF16)

        def layernorm_x(i):
            def piece(r):
                rows = pl.ds(pl.multiple_of(i * BLOCK + r, LN_ROWS), LN_ROWS)
                x = x_v[rows, :].astype(F32)
                d = x - jnp.sum(x, axis=1, keepdims=True) * (1.0 / dm)
                var = jnp.sum(d * d, axis=1, keepdims=True) * (1.0 / dm)
                xn = d * jax.lax.rsqrt(var + LN_EPS)
                for k in range(nd):
                    mix_v[xn_rows(k, i * BLOCK + r, LN_ROWS), :] = (
                        xn[:, k * LANES:(k + 1) * LANES])

            return [functools.partial(piece, r) for r in range(0, BLOCK, LN_ROWS)]

        win32 = win_v.bitcast(U32)

        def project_in(half, xn, store):
            def piece(lo, size):
                rows = pl.ds((half * fh + lo) // 2, size // 2)
                w = jnp.concatenate(
                    [pltpu.bitcast(win32[k, rows, :], BF16) for k in range(nd)], axis=1)
                store(lo, size, _dot(w, xn, NT))

            return [functools.partial(piece, lo, size) for lo, size in _chunks(fh, IN_ROWS[half])]

        def value_half(tile, xn):
            def store(lo, size, z):
                mix_v[z1_rows(tile, lo, size), :] = z

            return project_in(0, xn, store)

        def gate_half(k, xn):
            acc = {}

            def store(lo, size, z):
                z = _gelu(z)
                if lo == 0:
                    acc["pilot"] = jnp.sum(_fold_rows(z), axis=0, keepdims=True) * (1.0 / size)
                    acc["sum"] = acc["squares"] = 0.0
                d = z - acc["pilot"]
                z2t_v[k, pl.ds(lo, size), :] = d
                acc["sum"] += _fold_rows(d)
                acc["squares"] += _fold_rows(d * d)
                if lo + size == fh:
                    stat_v[k, 0] = acc["sum"]
                    stat_v[k, 1] = acc["squares"]

            return project_in(1, xn, store)

        def mixing_factors(group):
            mean, rstd = [], []
            for k in range(SIDE):
                mean.append(jnp.sum(stat_v[k, 0], axis=0, keepdims=True) * (1.0 / fh))
                var = jnp.sum(stat_v[k, 1], axis=0, keepdims=True) * (1.0 / fh) - mean[k] * mean[k]
                rstd.append(jax.lax.rsqrt(jnp.maximum(var, 0.0) + LN_EPS))

            def piece(lo):
                grid = [
                    [(z2t_v[k, pl.ds(r * fs + lo, 8), :] - mean[k]) * rstd[k] for k in range(SIDE)]
                    for r in range(SIDE)]
                for m, factor in enumerate(_strassen_left_factors(grid)):
                    mix_v[mixing_rows(m, group, lo, 8), :] = factor

            return [functools.partial(piece, lo) for lo in range(0, fs, 8)]

        early = groups // 2

        def phase1(i, carry):
            xn = [load_xn((i * SIDE + k) * LANES, LANES).astype(BF16) for k in range(SIDE)]
            _run(sum((gate_half(k, xn[k]) for k in range(SIDE)), []))

            pl.when(i == 0)(lambda: _wait(win_copies(0)))
            pl.when(i + 1 < groups)(lambda: x_copy(i + 1).wait())
            for c in range(early):
                pl.when(i == c)(lambda: _start(phase2_copies(c)))

            _run(_interleave(
                sum((value_half(i * SIDE + k, xn[k]) for k in range(SIDE)), []),
                _interleave(layernorm_x(jnp.minimum(i + 1, groups - 1)), mixing_factors(i))))
            return carry

        x_copy(0).wait()
        _start(win_copies(0))
        x_copy(1).start()
        _run(layernorm_x(0))
        for lo in range(0, LANES, 8):
            grid = [[mix_v[xn_rows(k, r * LANES + lo, 8), :] for k in range(SIDE)]
                    for r in range(SIDE)]
            for m, factor in enumerate(_strassen_left_factors(grid)):
                mix_v[ahead_rows(m, lo, 8), :] = factor
        _wait(win_copies(1))
        for i in range(2, groups):
            x_copy(i).start()
        mem_copy.start()
        with jax.named_scope("phase1"):
            jax.lax.fori_loop(0, groups, phase1, 0)

        def relayout_weights(i, part):
            parts = len(RELAYOUT_AFTER) + 3
            work = [(j, g, r) for j in range(3) for g in range(pair_chunk)
                    for r in range(0, dm // 2, RELAYOUT_ROWS)]
            for j, g, r in work[len(work) * part // parts:len(work) * (part + 1) // parts]:
                pair = i * pair_chunk + g
                a = wstage_v[j, pair, 0, pl.ds(r, RELAYOUT_ROWS), :]
                c = wstage_v[j, pair, 1, pl.ds(r, RELAYOUT_ROWS), :]
                words_v[w_rows(2 * pair * 3 + j, r, RELAYOUT_ROWS), :] = (
                    (a & jnp.uint32(0xFFFF)) | (c << 16))
                words_v[w_rows((2 * pair + 1) * 3 + j, r, RELAYOUT_ROWS), :] = (
                    (a >> 16) | (c & jnp.uint32(0xFFFF0000)))

        wsp32 = wsp_v.bitcast(U32)

        def mixing_block(group, k, c):
            rows = pl.ds(pl.multiple_of((group * SIDE + c) * (LANES // 2), LANES // 2), LANES // 2)
            return jnp.concatenate(
                [pltpu.bitcast(wsp32[g * SIDE + k, rows, :], BF16) for g in range(groups)], axis=1)

        def bias_row(tile):
            bias = bsp_v[...].astype(F32)
            pick = jax.lax.broadcasted_iota(jnp.int32, bias.shape, 0) == tile
            return jnp.sum(jnp.where(pick, bias, 0.0), axis=0, keepdims=True)

        def phase2(i, carry):
            for c in range(groups - early):
                pl.when(i == c)(lambda: _start(phase2_copies(c + early)))
            pl.when(i == groups - early)(lambda: _start(late_copies))
            _wait(phase2_copies(i))

            bias = [bias_row(i * SIDE + c) for c in range(SIDE)]
            issued = itertools.count(1)
            part = itertools.count()

            def product(m, rhs):
                lhs = jnp.concatenate(
                    [mix_v[mixing_rows(m, g, 0, fs), :] for g in range(groups)], axis=1)
                result = _dot(lhs, rhs.astype(BF16), NT)
                if next(issued) in RELAYOUT_AFTER:
                    words_v[zg_rows(i * SIDE, 0, 8), :] = pltpu.bitcast(result[:8], U32)
                    relayout_weights(i, next(part))
                return result

            def finished(blocks):
                for r, c, gate in blocks:
                    at = (i * SIDE + c, r * fs, fs)
                    zg = _gelu(mix_v[z1_rows(*at), :]) * (gate + bias[c])
                    words_v[zg_rows(*at), :] = pltpu.bitcast(zg, U32)
                relayout_weights(i, next(part))

            _strassen_multiply(
                MIX_ORDER, product,
                [[mixing_block(i, k, c) for c in range(SIDE)] for k in range(SIDE)], finished)
            return carry

        with jax.named_scope("phase2"):
            jax.lax.fori_loop(0, groups, phase2, 0)

    def recurrence(*rings):
        def ring_window(token, count):
            return pl.ds(pl.multiple_of((token + ring_rows - BLOCK) % ring_rows, 8), count)

        def phase3(i, carry):
            for j, first in itertools.product(range(3), range(0, RINGS, SIDE)):
                def weights(k, c):
                    rows = w_rows((i * RINGS + first + c) * 3 + j, k * (LANES // 2), LANES // 2)
                    return pltpu.bitcast(words_v[rows, :], BF16)

                rest = []
                issued = itertools.count()

                def product(m, rhs):
                    if next(issued) == REST_AFTER:
                        rest.extend(
                            sum(_dot(mix_v[xn_rows(k, 0, BLOCK), :], weights(k, c))
                                for k in range(SIDE, nd))
                            for c in range(SIDE))
                    return _dot(mix_v[ahead_rows(m, 0, LANES), :], rhs.astype(BF16))

                def finished(blocks):
                    for r, c, value in blocks:
                        rings[first + c][i * 3 + j, ring_window(r * LANES, LANES), :] = (
                            value + rest[c][r * LANES:(r + 1) * LANES])

                _strassen_multiply(
                    AHEAD_ORDER, product,
                    [[weights(k, c) for c in range(SIDE)] for k in range(SIDE)], finished)
            return carry

        with jax.named_scope("phase3"):
            jax.lax.fori_loop(0, heads // RINGS, phase3, 0)

        mem_copy.wait()
        _wait(late_copies)

        scale = dh ** -0.5
        qi = jax.lax.broadcasted_iota(jnp.int32, (mem_rows + seg, mem_rows + seg), 0)
        ki = jax.lax.broadcasted_iota(jnp.int32, (mem_rows + seg, mem_rows + seg), 1)
        mask = (qi < mem_rows) | (qi >= ki)
        wo32 = wo_v.bitcast(U32)
        wout32 = wout_v.bitcast(U32)

        def segment(s, mem):
            hid = jnp.concatenate([mem, load_xn(BLOCK + s * ride, ride)], axis=0).astype(BF16)
            put = ring_window(BLOCK + s * ride, ride)
            get = ring_window(s * seg, seg)

            def with_tokens(h, j, of_memory):
                return jnp.concatenate(
                    [of_memory, rings[h % RINGS][h // RINGS * 3 + j, get, :]], axis=0)

            acc = None
            live = {}
            for op, h in _head_schedule(heads):
                if op == "qkv":
                    w = jnp.concatenate(
                        [pltpu.bitcast(words_v[w_rows(h * 3 + j, 0, dm // 2), :], BF16)
                         for j in range(3)], axis=1)
                    r = _dot(hid, w)
                    for j in range(3):
                        rings[h % RINGS][h // RINGS * 3 + j, put, :] = (
                            r[mem_rows:, j * dh:(j + 1) * dh])
                    live[h] = [r[:mem_rows, j * dh:(j + 1) * dh] for j in range(3)]
                elif op == "scores":
                    q, k, v = live[h]
                    k = with_tokens(h, 1, k).astype(BF16)
                    live[h] = (_dot(with_tokens(h, 0, q), k, NT), v)
                elif op == "pv":
                    sc, v = live[h]
                    sc = jnp.where(mask, sc, MASK_VALUE / scale)
                    p = jnp.exp2((sc - jnp.max(sc, axis=1, keepdims=True)) * (scale * LOG2E))
                    total = jnp.sum(p, axis=1, keepdims=True)
                    live[h] = _dot(p, with_tokens(h, 2, v).astype(BF16)) * (1.0 / total)
                else:
                    rows = pl.ds(h * (dh // 2), dh // 2)
                    w = jnp.concatenate(
                        [pltpu.bitcast(wo32[n, rows, :], BF16) for n in range(nd)], axis=1)
                    y = _dot(live.pop(h), w)
                    acc = y if acc is None else acc + y
            return acc[:mem_rows], acc[mem_rows:]

        def out_copy(i):
            rows = pl.ds(pl.multiple_of(i * LANES, LANES), LANES)
            return pltpu.make_async_copy(out_v.at[rows], out_hbm.at[rows], sem_out.at[0])

        def phase4(i, mem):
            pl.when(i > 0)(lambda: out_copy(i - 1).start())

            zg = []
            for lo, size in _chunks(fh, LANES):
                t = pltpu.bitcast(words_v[zg_rows(i, lo, size), :], F32)
                if size < LANES:
                    t = jnp.concatenate([t, jnp.zeros((LANES - size, LANES), F32)], axis=0)
                zg.append(t.T)
            zg = jnp.concatenate(zg, axis=1)

            attended, gates = [], []
            for u in range(LANES // seg):
                mem, tokens = segment(i * (LANES // seg) + u, mem)
                attended.append(tokens)
                if u + 1 < len(GATE_ROWS):
                    w = jnp.concatenate(
                        [pltpu.bitcast(wout32[n], BF16) for n in range(nd)], axis=1)
                    y = _dot(zg[GATE_ROWS[u]:GATE_ROWS[u + 1]], w)
                    gates.append(y * jax.nn.sigmoid(y))
            rows = pl.ds(pl.multiple_of(i * LANES, LANES), LANES)
            gated = jnp.concatenate(attended, axis=0) * jnp.concatenate(gates, axis=0)
            out_v[rows, :] = (x_v[rows, :].astype(F32) + gated).astype(BF16)
            return mem

        with jax.named_scope("phase4"):
            jax.lax.fori_loop(0, tiles, phase4, mem_v[...].astype(F32))
        out_copy(tiles - 1).start()
        pltpu.make_async_copy(out_v, out_hbm, sem_out.at[0]).wait()

    pl.run_scoped(
        gmlp,
        pltpu.VMEM((tiles, LANES), BF16),
        pltpu.VMEM((nd, 2 * fh, LANES), BF16),
        pltpu.VMEM((tiles, seq, LANES), BF16),
        pltpu.VMEM((3, heads // 2, 2, dm // 2, dh), U32),
        pltpu.VMEM((SIDE, 2, 8, LANES), F32),
        pltpu.VMEM((SIDE, fh, LANES), F32),
    )
    pl.run_scoped(recurrence, *[pltpu.VMEM((heads // RINGS * 3, ring_rows, dh), F32)] * RINGS)


@functools.partial(jax.jit, static_argnames=("A_seg_len",))
def pallas_recurrent_scan__memory_aug_recurrent_mem_tr__mixer_gmlp__prompt_kernel(
    A_x: jax.Array,
    A_mem0: jax.Array,
    A_Wq: jax.Array,
    A_Wk: jax.Array,
    A_Wv: jax.Array,
    A_Wo: jax.Array,
    A_seg_len: int,
    B_x: jax.Array,
    B_w_in: jax.Array,
    B_w_sp: jax.Array,
    B_b_sp: jax.Array,
    B_w_out: jax.Array,
):
    del B_x
    batch, seq, dm = A_x.shape
    heads, dh = A_Wq.shape[1], A_Wq.shape[2]
    mem_rows = A_mem0.shape[1]
    seg = A_seg_len
    fh = B_w_in.shape[1] // 2
    nd, nf, tiles, groups = dm // LANES, pl.cdiv(fh, LANES), seq // LANES, seq // BLOCK
    assert batch == 1 and dh == LANES and dm % LANES == 0 and nd > SIDE
    assert seq % BLOCK == 0 and groups >= 4 and heads % (2 * groups) == 0 and heads % RINGS == 0
    assert fh % 16 == 0 and fh % (8 * SIDE) == 0 and dm % (2 * RELAYOUT_ROWS) == 0
    assert mem_rows % 8 == 0 and seg % (8 * groups) == 0 and LANES // seg >= len(GATE_ROWS)

    hbm = pl.BlockSpec(memory_space=pltpu.MemorySpace.HBM)
    dma = pltpu.SemaphoreType.DMA
    out = pl.pallas_call(
        functools.partial(
            _kernel, seq=seq, dm=dm, heads=heads, dh=dh, mem_rows=mem_rows, seg=seg, fh=fh),
        out_shape=jax.ShapeDtypeStruct((seq, dm), BF16),
        in_specs=[hbm] * 10,
        out_specs=hbm,
        scratch_shapes=[
            pltpu.VMEM((seq, dm), BF16),
            pltpu.VMEM((mem_rows, dm), BF16),
            pltpu.VMEM((nd, nf * LANES, LANES), BF16),
            pltpu.VMEM((nd, heads * dh, LANES), BF16),
            pltpu.VMEM((heads * 3 * dm // 2 + tiles * fh, LANES), U32),
            pltpu.VMEM(
                (nd * seq + tiles * fh + PRODUCTS * (groups * fh // SIDE + LANES), LANES), F32),
            pltpu.VMEM((seq, dm), BF16),
            dma((groups,)), dma((2,)), dma((2,)), dma((groups,)), dma((1,)), dma((1,)),
        ],
        compiler_params=pltpu.CompilerParams(
            vmem_limit_bytes=116 * 1024 * 1024,
            flags={"XLA_TPU_EVENLY_DISTRIBUTE_CRITICAL_NODES": True}),
    )(
        A_x.reshape(seq, dm),
        A_mem0.reshape(mem_rows, dm),
        A_Wq.reshape(dm // 2, 2, heads, dh),
        A_Wk.reshape(dm // 2, 2, heads, dh),
        A_Wv.reshape(dm // 2, 2, heads, dh),
        A_Wo.reshape(heads * dh, dm),
        B_w_in.T,
        B_w_sp,
        B_b_sp.reshape(tiles, LANES),
        B_w_out,
    )
    return out.reshape(batch, seq, dm)
```

```python
import functools
import itertools
import math

import jax
import jax.numpy as jnp
import jax.experimental.pallas as pl
import jax.experimental.pallas.tpu as pltpu

F32 = jnp.float32
BF16 = jnp.bfloat16
U32 = jnp.uint32

LANES = 128
LN_EPS = 1e-5
LOG2E = 1.4426950408889634
MASK_VALUE = -1000000000.0
GELU_C1 = 0.7978845608028654
GELU_C2 = 0.044715 * GELU_C1

NN = (((1,), (0,)), ((), ()))
NT = (((1,), (1,)), ((), ()))

STRASSEN_LHS = (
    ((0, 0, 1), (1, 1, 1)), ((1, 0, 1), (1, 1, 1)), ((0, 0, 1),), ((1, 1, 1),),
    ((0, 0, 1), (0, 1, 1)), ((1, 0, 1), (0, 0, -1)), ((0, 1, 1), (1, 1, -1)))
STRASSEN_RHS = (
    ((0, 0, 1), (1, 1, 1)), ((0, 0, 1),), ((0, 1, 1), (1, 1, -1)), ((1, 0, 1), (0, 0, -1)),
    ((1, 1, 1),), ((0, 0, 1), (0, 1, 1)), ((1, 0, 1), (1, 1, 1)))
STRASSEN_OUT = (
    (((0, 1), (3, 1), (4, -1), (6, 1)), ((2, 1), (4, 1))),
    (((1, 1), (3, 1)), ((0, 1), (1, -1), (2, 1), (5, 1))))
SIDE = 4
PRODUCTS = 49
BLOCK = SIDE * LANES

LN_ROWS = 64
IN_ROWS = (80, 96)
MIX_ORDER = ((1, 4, 3, 0, 6, 2, 5), (4, 0, 1, 3, 6, 2, 5))
AHEAD_ORDER = ((1, 4, 3, 6, 0, 5, 2), (4, 0, 1, 3, 6, 5, 2))
REST_AFTER = 7
RELAYOUT_AFTER = (2, 9, 16)
RELAYOUT_ROWS = 64
RINGS = 8
LAG_SCORES, LAG_PV = 3, 6
FIRST_OUT, OUT_PERIOD, LAST_OUTS = 17, 2, (2, 3, 3, 3, 4, 3)
GATE_ROWS = (0, 48, 80, LANES)


def _dot(a, b, dims=NN):
    return jax.lax.dot_general(a, b, dims, preferred_element_type=F32)


def _gelu(x):
    t = jnp.tanh(x * (GELU_C1 + GELU_C2 * (x * x)))
    hx = 0.5 * x
    return hx + hx * t


def _chunks(total, size):
    return [(lo, min(size, total - lo)) for lo in range(0, total, size)]


def _fold_rows(x):
    return functools.reduce(lambda a, b: a + b, [x[r:r + 8] for r in range(0, x.shape[0], 8)])


def _interleave(main, side):
    merged, done = [], 0
    for k, item in enumerate(main):
        upto = len(side) * (k + 1) // len(main)
        merged += [item] + side[done:upto]
        done = upto
    return merged


def _run(thunks):
    for fn in thunks:
        fn()


def _start(copies):
    for cp in copies:
        cp.start()


def _wait(copies):
    for cp in copies:
        cp.wait()


def _signed_sum(terms):
    total = terms[0][0]
    for value, sign in terms[1:]:
        total, value = total.astype(F32), value.astype(F32)
        total = total + value if sign > 0 else total - value
    return total


def _strassen_factor(terms, grid):
    half = len(grid) // 2
    return [
        [_signed_sum([(grid[r * half + a][c * half + b], sign) for r, c, sign in terms])
         for b in range(half)] for a in range(half)]


def _strassen_left_factors(grid):
    if len(grid) == 1:
        return [grid[0][0]]
    return sum((_strassen_left_factors(_strassen_factor(t, grid)) for t in STRASSEN_LHS), [])


def _strassen_multiply(order, product, right, finished=None, index=0):
    half = len(right) // 2
    if not half:
        return [[product(index, right[0][0])]]
    grid = [[None] * (2 * half) for _ in range(2 * half)]
    for k, m in enumerate(order[0]):
        inner = _strassen_multiply(
            order[1:], product, _strassen_factor(STRASSEN_RHS[m], right), None, index * 7 + m)
        for r, c in itertools.product(range(2), range(2)):
            for sign in [sign for q, sign in STRASSEN_OUT[r][c] if q == m]:
                cells = [(r * half + a, c * half + b, inner[a][b])
                         for a in range(half) for b in range(half)]
                for row, col, new in cells:
                    old = grid[row][col]
                    if old is None:
                        grid[row][col] = new if sign > 0 else -new
                    else:
                        grid[row][col] = old + new if sign > 0 else old - new
                if finished and all(q in order[0][:k + 1] for q, _ in STRASSEN_OUT[r][c]):
                    finished([(row, col, grid[row][col]) for row, col, _ in cells])
    return grid


def _head_schedule(heads):
    ops = []
    out = 0
    for t in range(heads + LAG_PV):
        if t < heads:
            count = int(t >= FIRST_OUT and (t - FIRST_OUT) % OUT_PERIOD == 0)
        else:
            count = LAST_OUTS[t - heads]
        for _ in range(count):
            if out < t - LAG_PV:
                ops.append(("out", out))
                out += 1
        if t < heads:
            ops.append(("qkv", t))
        if 0 <= t - LAG_SCORES < heads:
            ops.append(("scores", t - LAG_SCORES))
        if t >= LAG_PV:
            ops.append(("pv", t - LAG_PV))
    return ops + [("out", h) for h in range(out, heads)]


def _kernel(
    x_hbm, mem_hbm, wq_hbm, wk_hbm, wv_hbm, wo_hbm, win_hbm, wsp_hbm, bsp_hbm, wout_hbm,
    out_hbm,
    x_v, mem_v, wout_v, wo_v, words_v, mix_v, out_v,
    sem_x, sem_small, sem_win, sem_w, sem_wo, sem_out,
    *, seq, dm, heads, dh, mem_rows, seg, fh,
):
    nd = dm // LANES
    nf = pl.cdiv(fh, LANES)
    tiles = seq // LANES
    groups = seq // BLOCK
    fs = fh // SIDE
    pair_chunk = heads // 2 // groups
    ride = seg - BLOCK * seg // seq
    ring_rows = pl.cdiv(BLOCK + ride, math.lcm(seg, ride)) * math.lcm(seg, ride)

    def xn_rows(k, first, count):
        return pl.ds(pl.multiple_of(k * seq + first, 8), count)

    def z1_rows(tile, lo, size):
        return pl.ds(pl.multiple_of(nd * seq + tile * fh + lo, 8), size)

    def mixing_rows(product, group, lo, size):
        first = nd * seq + tiles * fh + (product * groups + group) * fs + lo
        return pl.ds(pl.multiple_of(first, 8), size)

    def ahead_rows(product, lo, size):
        return pl.ds(nd * seq + tiles * fh + PRODUCTS * groups * fs + product * LANES + lo, size)

    def w_rows(tile, lo, size):
        return pl.ds(pl.multiple_of(tile * (dm // 2) + lo, 8), size)

    def zg_rows(tile, lo, size):
        return pl.ds(pl.multiple_of(heads * 3 * (dm // 2) + tile * fh + lo, 8), size)

    def load_xn(first, count):
        return jnp.concatenate([mix_v[xn_rows(k, first, count), :] for k in range(nd)], axis=1)

    mem_copy = pltpu.make_async_copy(mem_hbm, mem_v, sem_small.at[0])
    late_copies = [
        pltpu.make_async_copy(
            wout_hbm.at[:, pl.ds(n * LANES, LANES)], wout_v.at[n, pl.ds(0, fh)], sem_wo.at[0])
        for n in range(nd)
    ] + [
        pltpu.make_async_copy(wo_hbm.at[:, pl.ds(n * LANES, LANES)], wo_v.at[n], sem_wo.at[0])
        for n in range(nd)
    ]

    def gmlp(bsp_v, win_v, wsp_v, wstage_v, stat_v, z2t_v):
        def x_copy(i):
            rows = pl.ds(pl.multiple_of(i * BLOCK, BLOCK), BLOCK)
            return pltpu.make_async_copy(x_hbm.at[rows], x_v.at[rows], sem_x.at[i])

        def win_copies(half):
            rows = pl.ds(half * fh, fh)
            return [
                pltpu.make_async_copy(
                    win_hbm.at[rows, pl.ds(k * LANES, LANES)], win_v.at[k, rows], sem_win.at[half])
                for k in range(nd)
            ]

        def phase2_copies(i):
            rows = pl.ds(pl.multiple_of(i * BLOCK, BLOCK), BLOCK)
            return [
                pltpu.make_async_copy(
                    wsp_hbm.at[rows, pl.ds(k * LANES, LANES)], wsp_v.at[k, rows], sem_w.at[i])
                for k in range(tiles)
            ] + [
                pltpu.make_async_copy(
                    src.bitcast(U32).at[:, odd, i * pair_chunk + g],
                    wstage_v.at[j, i * pair_chunk + g, odd], sem_w.at[i])
                for j, src in enumerate((wq_hbm, wk_hbm, wv_hbm))
                for g in range(pair_chunk) for odd in range(2)
            ]

        bsp_copy = pltpu.make_async_copy(bsp_hbm, bsp_v, sem_small.at[1])
        bsp_copy.start()
        x_copy(0).start()
        bsp_copy.wait()
        _start(win_copies(1))

        if nf * LANES > fh:
            wout_v[:, pl.ds(fh, nf * LANES - fh), :] = jnp.zeros(
                (nd, nf * LANES - fh, LANES), BF16)

        def layernorm_x(i):
            def piece(r):
                rows = pl.ds(pl.multiple_of(i * BLOCK + r, LN_ROWS), LN_ROWS)
                x = x_v[rows, :].astype(F32)
                d = x - jnp.sum(x, axis=1, keepdims=True) * (1.0 / dm)
                var = jnp.sum(d * d, axis=1, keepdims=True) * (1.0 / dm)
                xn = d * jax.lax.rsqrt(var + LN_EPS)
                for k in range(nd):
                    mix_v[xn_rows(k, i * BLOCK + r, LN_ROWS), :] = (
                        xn[:, k * LANES:(k + 1) * LANES])

            return [functools.partial(piece, r) for r in range(0, BLOCK, LN_ROWS)]

        win32 = win_v.bitcast(U32)

        def project_in(half, xn, store):
            def piece(lo, size):
                rows = pl.ds((half * fh + lo) // 2, size // 2)
                w = jnp.concatenate(
                    [pltpu.bitcast(win32[k, rows, :], BF16) for k in range(nd)], axis=1)
                store(lo, size, _dot(w, xn, NT))

            return [functools.partial(piece, lo, size) for lo, size in _chunks(fh, IN_ROWS[half])]

        def value_half(tile, xn):
            def store(lo, size, z):
                mix_v[z1_rows(tile, lo, size), :] = z

            return project_in(0, xn, store)

        def gate_half(k, xn):
            acc = {}

            def store(lo, size, z):
                z = _gelu(z)
                if lo == 0:
                    acc["pilot"] = jnp.sum(_fold_rows(z), axis=0, keepdims=True) * (1.0 / size)
                    acc["sum"] = acc["squares"] = 0.0
                d = z - acc["pilot"]
                z2t_v[k, pl.ds(lo, size), :] = d
                acc["sum"] += _fold_rows(d)
                acc["squares"] += _fold_rows(d * d)
                if lo + size == fh:
                    stat_v[k, 0] = acc["sum"]
                    stat_v[k, 1] = acc["squares"]

            return project_in(1, xn, store)

        def mixing_factors(group):
            mean, rstd = [], []
            for k in range(SIDE):
                mean.append(jnp.sum(stat_v[k, 0], axis=0, keepdims=True) * (1.0 / fh))
                var = jnp.sum(stat_v[k, 1], axis=0, keepdims=True) * (1.0 / fh) - mean[k] * mean[k]
                rstd.append(jax.lax.rsqrt(jnp.maximum(var, 0.0) + LN_EPS))

            def piece(lo):
                grid = [
                    [(z2t_v[k, pl.ds(r * fs + lo, 8), :] - mean[k]) * rstd[k] for k in range(SIDE)]
                    for r in range(SIDE)]
                for m, factor in enumerate(_strassen_left_factors(grid)):
                    mix_v[mixing_rows(m, group, lo, 8), :] = factor

            return [functools.partial(piece, lo) for lo in range(0, fs, 8)]

        early = groups // 2

        def phase1(i, carry):
            xn = [load_xn((i * SIDE + k) * LANES, LANES).astype(BF16) for k in range(SIDE)]
            _run(sum((gate_half(k, xn[k]) for k in range(SIDE)), []))

            pl.when(i == 0)(lambda: _wait(win_copies(0)))
            pl.when(i + 1 < groups)(lambda: x_copy(i + 1).wait())
            for c in range(early):
                pl.when(i == c)(lambda: _start(phase2_copies(c)))

            _run(_interleave(
                sum((value_half(i * SIDE + k, xn[k]) for k in range(SIDE)), []),
                _interleave(layernorm_x(jnp.minimum(i + 1, groups - 1)), mixing_factors(i))))
            return carry

        x_copy(0).wait()
        _start(win_copies(0))
        x_copy(1).start()
        _run(layernorm_x(0))
        for lo in range(0, LANES, 8):
            grid = [[mix_v[xn_rows(k, r * LANES + lo, 8), :] for k in range(SIDE)]
                    for r in range(SIDE)]
            for m, factor in enumerate(_strassen_left_factors(grid)):
                mix_v[ahead_rows(m, lo, 8), :] = factor
        _wait(win_copies(1))
        for i in range(2, groups):
            x_copy(i).start()
        mem_copy.start()
        jax.lax.fori_loop(0, groups, phase1, 0)

        def relayout_weights(i, part):
            parts = len(RELAYOUT_AFTER) + 3
            work = [(j, g, r) for j in range(3) for g in range(pair_chunk)
                    for r in range(0, dm // 2, RELAYOUT_ROWS)]
            for j, g, r in work[len(work) * part // parts:len(work) * (part + 1) // parts]:
                pair = i * pair_chunk + g
                a = wstage_v[j, pair, 0, pl.ds(r, RELAYOUT_ROWS), :]
                c = wstage_v[j, pair, 1, pl.ds(r, RELAYOUT_ROWS), :]
                words_v[w_rows(2 * pair * 3 + j, r, RELAYOUT_ROWS), :] = (
                    (a & jnp.uint32(0xFFFF)) | (c << 16))
                words_v[w_rows((2 * pair + 1) * 3 + j, r, RELAYOUT_ROWS), :] = (
                    (a >> 16) | (c & jnp.uint32(0xFFFF0000)))

        wsp32 = wsp_v.bitcast(U32)

        def mixing_block(group, k, c):
            rows = pl.ds(pl.multiple_of((group * SIDE + c) * (LANES // 2), LANES // 2), LANES // 2)
            return jnp.concatenate(
                [pltpu.bitcast(wsp32[g * SIDE + k, rows, :], BF16) for g in range(groups)], axis=1)

        def bias_row(tile):
            bias = bsp_v[...].astype(F32)
            pick = jax.lax.broadcasted_iota(jnp.int32, bias.shape, 0) == tile
            return jnp.sum(jnp.where(pick, bias, 0.0), axis=0, keepdims=True)

        def phase2(i, carry):
            for c in range(groups - early):
                pl.when(i == c)(lambda: _start(phase2_copies(c + early)))
            pl.when(i == groups - early)(lambda: _start(late_copies))
            _wait(phase2_copies(i))

            bias = [bias_row(i * SIDE + c) for c in range(SIDE)]
            issued = itertools.count(1)
            part = itertools.count()

            def product(m, rhs):
                lhs = jnp.concatenate(
                    [mix_v[mixing_rows(m, g, 0, fs), :] for g in range(groups)], axis=1)
                result = _dot(lhs, rhs.astype(BF16), NT)
                if next(issued) in RELAYOUT_AFTER:
                    words_v[zg_rows(i * SIDE, 0, 8), :] = pltpu.bitcast(result[:8], U32)
                    relayout_weights(i, next(part))
                return result

            def finished(blocks):
                for r, c, gate in blocks:
                    at = (i * SIDE + c, r * fs, fs)
                    zg = _gelu(mix_v[z1_rows(*at), :]) * (gate + bias[c])
                    words_v[zg_rows(*at), :] = pltpu.bitcast(zg, U32)
                relayout_weights(i, next(part))

            _strassen_multiply(
                MIX_ORDER, product,
                [[mixing_block(i, k, c) for c in range(SIDE)] for k in range(SIDE)], finished)
            return carry

        jax.lax.fori_loop(0, groups, phase2, 0)

    def recurrence(*rings):
        def ring_window(token, count):
            return pl.ds(pl.multiple_of((token + ring_rows - BLOCK) % ring_rows, 8), count)

        def phase3(i, carry):
            for j, first in itertools.product(range(3), range(0, RINGS, SIDE)):
                def weights(k, c):
                    rows = w_rows((i * RINGS + first + c) * 3 + j, k * (LANES // 2), LANES // 2)
                    return pltpu.bitcast(words_v[rows, :], BF16)

                rest = []
                issued = itertools.count()

                def product(m, rhs):
                    if next(issued) == REST_AFTER:
                        rest.extend(
                            sum(_dot(mix_v[xn_rows(k, 0, BLOCK), :], weights(k, c))
                                for k in range(SIDE, nd))
                            for c in range(SIDE))
                    return _dot(mix_v[ahead_rows(m, 0, LANES), :], rhs.astype(BF16))

                def finished(blocks):
                    for r, c, value in blocks:
                        rings[first + c][i * 3 + j, ring_window(r * LANES, LANES), :] = (
                            value + rest[c][r * LANES:(r + 1) * LANES])

                _strassen_multiply(
                    AHEAD_ORDER, product,
                    [[weights(k, c) for c in range(SIDE)] for k in range(SIDE)], finished)
            return carry

        jax.lax.fori_loop(0, heads // RINGS, phase3, 0)

        mem_copy.wait()
        _wait(late_copies)

        scale = dh ** -0.5
        qi = jax.lax.broadcasted_iota(jnp.int32, (mem_rows + seg, mem_rows + seg), 0)
        ki = jax.lax.broadcasted_iota(jnp.int32, (mem_rows + seg, mem_rows + seg), 1)
        mask = (qi < mem_rows) | (qi >= ki)
        wo32 = wo_v.bitcast(U32)
        wout32 = wout_v.bitcast(U32)

        def segment(s, mem):
            hid = jnp.concatenate([mem, load_xn(BLOCK + s * ride, ride)], axis=0).astype(BF16)
            put = ring_window(BLOCK + s * ride, ride)
            get = ring_window(s * seg, seg)

            def with_tokens(h, j, of_memory):
                return jnp.concatenate(
                    [of_memory, rings[h % RINGS][h // RINGS * 3 + j, get, :]], axis=0)

            acc = None
            live = {}
            for op, h in _head_schedule(heads):
                if op == "qkv":
                    w = jnp.concatenate(
                        [pltpu.bitcast(words_v[w_rows(h * 3 + j, 0, dm // 2), :], BF16)
                         for j in range(3)], axis=1)
                    r = _dot(hid, w)
                    for j in range(3):
                        rings[h % RINGS][h // RINGS * 3 + j, put, :] = (
                            r[mem_rows:, j * dh:(j + 1) * dh])
                    live[h] = [r[:mem_rows, j * dh:(j + 1) * dh] for j in range(3)]
                elif op == "scores":
                    q, k, v = live[h]
                    k = with_tokens(h, 1, k).astype(BF16)
                    live[h] = (_dot(with_tokens(h, 0, q), k, NT), v)
                elif op == "pv":
                    sc, v = live[h]
                    sc = jnp.where(mask, sc, MASK_VALUE / scale)
                    p = jnp.exp2((sc - jnp.max(sc, axis=1, keepdims=True)) * (scale * LOG2E))
                    total = jnp.sum(p, axis=1, keepdims=True)
                    live[h] = _dot(p, with_tokens(h, 2, v).astype(BF16)) * (1.0 / total)
                else:
                    rows = pl.ds(h * (dh // 2), dh // 2)
                    w = jnp.concatenate(
                        [pltpu.bitcast(wo32[n, rows, :], BF16) for n in range(nd)], axis=1)
                    y = _dot(live.pop(h), w)
                    acc = y if acc is None else acc + y
            return acc[:mem_rows], acc[mem_rows:]

        def out_copy(i):
            rows = pl.ds(pl.multiple_of(i * LANES, LANES), LANES)
            return pltpu.make_async_copy(out_v.at[rows], out_hbm.at[rows], sem_out.at[0])

        def phase4(i, mem):
            zg = []
            for lo, size in _chunks(fh, LANES):
                t = pltpu.bitcast(words_v[zg_rows(i, lo, size), :], F32)
                if size < LANES:
                    t = jnp.concatenate([t, jnp.zeros((LANES - size, LANES), F32)], axis=0)
                zg.append(t.T)
            zg = jnp.concatenate(zg, axis=1)

            attended, gates = [], []
            for u in range(LANES // seg):
                mem, tokens = segment(i * (LANES // seg) + u, mem)
                attended.append(tokens)
                if u == 0:
                    pl.when(i > 0)(lambda: out_copy(i - 1).start())
                if u + 1 < len(GATE_ROWS):
                    w = jnp.concatenate(
                        [pltpu.bitcast(wout32[n], BF16) for n in range(nd)], axis=1)
                    y = _dot(zg[GATE_ROWS[u]:GATE_ROWS[u + 1]], w)
                    gates.append(y * jax.nn.sigmoid(y))
            rows = pl.ds(pl.multiple_of(i * LANES, LANES), LANES)
            gated = jnp.concatenate(attended, axis=0) * jnp.concatenate(gates, axis=0)
            out_v[rows, :] = (x_v[rows, :].astype(F32) + gated).astype(BF16)
            return mem

        jax.lax.fori_loop(0, tiles, phase4, mem_v[...].astype(F32))
        out_copy(tiles - 1).start()
        pltpu.make_async_copy(out_v, out_hbm, sem_out.at[0]).wait()

    pl.run_scoped(
        gmlp,
        pltpu.VMEM((tiles, LANES), BF16),
        pltpu.VMEM((nd, 2 * fh, LANES), BF16),
        pltpu.VMEM((tiles, seq, LANES), BF16),
        pltpu.VMEM((3, heads // 2, 2, dm // 2, dh), U32),
        pltpu.VMEM((SIDE, 2, 8, LANES), F32),
        pltpu.VMEM((SIDE, fh, LANES), F32),
    )
    pl.run_scoped(recurrence, *[pltpu.VMEM((heads // RINGS * 3, ring_rows, dh), F32)] * RINGS)


@functools.partial(jax.jit, static_argnames=("A_seg_len",))
def pallas_recurrent_scan__memory_aug_recurrent_mem_tr__mixer_gmlp__prompt_kernel(
    A_x: jax.Array,
    A_mem0: jax.Array,
    A_Wq: jax.Array,
    A_Wk: jax.Array,
    A_Wv: jax.Array,
    A_Wo: jax.Array,
    A_seg_len: int,
    B_x: jax.Array,
    B_w_in: jax.Array,
    B_w_sp: jax.Array,
    B_b_sp: jax.Array,
    B_w_out: jax.Array,
):
    del B_x
    batch, seq, dm = A_x.shape
    heads, dh = A_Wq.shape[1], A_Wq.shape[2]
    mem_rows = A_mem0.shape[1]
    seg = A_seg_len
    fh = B_w_in.shape[1] // 2
    nd, nf, tiles, groups = dm // LANES, pl.cdiv(fh, LANES), seq // LANES, seq // BLOCK
    assert batch == 1 and dh == LANES and dm % LANES == 0 and nd > SIDE
    assert seq % BLOCK == 0 and groups >= 4 and heads % (2 * groups) == 0 and heads % RINGS == 0
    assert fh % 16 == 0 and fh % (8 * SIDE) == 0 and dm % (2 * RELAYOUT_ROWS) == 0
    assert mem_rows % 8 == 0 and seg % (8 * groups) == 0 and LANES // seg >= len(GATE_ROWS)

    hbm = pl.BlockSpec(memory_space=pltpu.MemorySpace.HBM)
    dma = pltpu.SemaphoreType.DMA
    out = pl.pallas_call(
        functools.partial(
            _kernel, seq=seq, dm=dm, heads=heads, dh=dh, mem_rows=mem_rows, seg=seg, fh=fh),
        out_shape=jax.ShapeDtypeStruct((seq, dm), BF16),
        in_specs=[hbm] * 10,
        out_specs=hbm,
        scratch_shapes=[
            pltpu.VMEM((seq, dm), BF16),
            pltpu.VMEM((mem_rows, dm), BF16),
            pltpu.VMEM((nd, nf * LANES, LANES), BF16),
            pltpu.VMEM((nd, heads * dh, LANES), BF16),
            pltpu.VMEM((heads * 3 * dm // 2 + tiles * fh, LANES), U32),
            pltpu.VMEM(
                (nd * seq + tiles * fh + PRODUCTS * (groups * fh // SIDE + LANES), LANES), F32),
            pltpu.VMEM((seq, dm), BF16),
            dma((groups,)), dma((2,)), dma((2,)), dma((groups,)), dma((1,)), dma((1,)),
        ],
        compiler_params=pltpu.CompilerParams(
            vmem_limit_bytes=116 * 1024 * 1024,
            flags={"XLA_TPU_EVENLY_DISTRIBUTE_CRITICAL_NODES": True}),
    )(
        A_x.reshape(seq, dm),
        A_mem0.reshape(mem_rows, dm),
        A_Wq.reshape(dm // 2, 2, heads, dh),
        A_Wk.reshape(dm // 2, 2, heads, dh),
        A_Wv.reshape(dm // 2, 2, heads, dh),
        A_Wo.reshape(heads * dh, dm),
        B_w_in.T,
        B_w_sp,
        B_b_sp.reshape(tiles, LANES),
        B_w_out,
    )
    return out.reshape(batch, seq, dm)
```
